```python
import os as _os
_os.environ.setdefault("JAX_PLATFORMS", "cpu")
import jax
import jax.numpy as jnp

def _softmax(x, axis=-1):
    return jax.nn.softmax(x, axis=axis)
def _gelu(x):
    return jax.nn.gelu(x, approximate=True)
def _silu(x):
    return jax.nn.silu(x)
def _sigmoid(x):
    return jax.nn.sigmoid(x)
def _layernorm(x, axis=-1, eps=1e-5):
    m = jnp.mean(x, axis=axis, keepdims=True)
    v = jnp.var(x, axis=axis, keepdims=True)
    return (x - m) / jnp.sqrt(v + eps)
def _scatter_add(tgt, idx, src, axis=0):
    return tgt.at[idx].add(src)
def _segment_sum(src, seg, n):
    return jax.ops.segment_sum(src, seg, n)
class _Rng:
    def __init__(self, key):
        self._k = key
    def _next(self):
        self._k, sub = jax.random.split(self._k)
        return sub
    def normal(self, shape):
        return jax.random.normal(self._next(), shape, dtype=jnp.bfloat16)
    def randint(self, lo, hi, shape):
        return jax.random.randint(self._next(), shape, lo, hi, dtype=jnp.int32)
    def uniform(self, shape, lo=0.0, hi=1.0):
        return jax.random.uniform(self._next(), shape, jnp.bfloat16, lo, hi)
    def permutation(self, n):
        return jax.random.permutation(self._next(), n)


kernel_name = 'standalone__linear_kernel_rfa__decode'

def setup_inputs():
    _rng = _Rng(jax.random.key(int.from_bytes(__import__("os").urandom(4), "little")))
    _w = (lambda a: (lambda t: t.astype(jnp.bfloat16) if jnp.issubdtype(t.dtype, jnp.floating) else t)(jnp.asarray(a)))
    B, H, Sq, Sk, D, M = 2, 16, 1, 16384, 256, 16
    return {
        "q": _w((lambda *s: _rng.normal(s) * 0.4)(B, H, Sq, D)),
        "k": _w((lambda *s: _rng.normal(s) * 1.6)(B, H, Sk, D)),
        "v": _w((lambda *s: _rng.normal(s) * 1.6)(B, H, Sk, D)),
        "omega": _w((lambda *s: _rng.normal(s) * 1.6)(M, D)),
    }

def reference(q, k, v, omega):
    d = q.shape[-1]
    m = omega.shape[0]
    scale = float(d) ** -0.25
    qs = q * scale
    ks = k * scale
    q_proj = jnp.einsum("bhsd,md->bhsm", qs, omega)
    k_proj = jnp.einsum("bhsd,md->bhsm", ks, omega)
    q_sq = 0.5 * jnp.einsum("bhsd,bhsd->bhs", qs, qs)[..., None]
    k_sq = 0.5 * jnp.einsum("bhsd,bhsd->bhs", ks, ks)[..., None]
    inv_sqrt_m = float(m) ** -0.5
    phi_q = jnp.exp(q_proj - q_sq) * inv_sqrt_m + 1e-6
    phi_k = jnp.exp(k_proj - k_sq) * inv_sqrt_m + 1e-6
    kv = jnp.einsum("bhsm,bhsd->bhmd", phi_k, v)
    z  = jnp.einsum("bhsm->bhm", phi_k)
    num = jnp.einsum("bhqm,bhmd->bhqd", phi_q, kv)
    den = jnp.einsum("bhqm,bhm->bhq", phi_q, z)[..., None] + 1e-6
    return num / den
```

```python
import functools

import jax
import jax.numpy as jnp
from jax import lax
import jax.experimental.pallas as pl
import jax.experimental.pallas.tpu as pltpu

_NT = (((1,), (1,)), ((), ()))

_CHUNK = 1024
_SLOTS = 4
_DMA_ROWS = 64


def _kernel(q_hbm, om_hbm, k_hbm, v_hbm, o_ref,
            kb, vb, qb, omb, kv_acc, z_acc, sems, sem_in, *, sk):
    n_rows, d = k_hbm.shape
    m = omb.shape[0]
    scale = float(d) ** -0.25
    inv_sqrt_m = float(m) ** -0.5
    n_chunks = n_rows // _CHUNK
    per_head = sk // _CHUNK

    def start(i, slot):
        for s in range(_CHUNK // _DMA_ROWS):
            src = pl.ds(i * _CHUNK + s * _DMA_ROWS, _DMA_ROWS)
            dst = pl.ds(s * _DMA_ROWS, _DMA_ROWS)
            pltpu.make_async_copy(
                k_hbm.at[src], kb.at[slot, dst], sems.at[0, slot]).start(priority=0)
            pltpu.make_async_copy(
                v_hbm.at[src], vb.at[slot, dst], sems.at[1, slot]).start(priority=1)

    def wait(buf, which, slot):
        pltpu.make_async_copy(buf.at[slot], buf.at[slot], sems.at[which, slot]).wait()

    for i in range(_SLOTS - 1):
        start(i, i)
    om_copy = pltpu.make_async_copy(om_hbm, omb, sem_in.at[0])
    q_copy = pltpu.make_async_copy(q_hbm, qb, sem_in.at[1])
    om_copy.start()
    q_copy.start()
    kv_acc[...] = jnp.zeros_like(kv_acc)
    z_acc[...] = jnp.zeros_like(z_acc)
    om_copy.wait()
    q_copy.wait()

    def phi_k(k):
        proj = lax.dot_general(omb[...], k, _NT, preferred_element_type=jnp.float32)
        lo = k[:, : d // 2].astype(jnp.float32)
        hi = k[:, d // 2:].astype(jnp.float32)
        sq = (lo * lo + hi * hi).astype(jnp.bfloat16)
        ones = jnp.ones((m, d // 2), jnp.bfloat16)
        ssq = lax.dot_general(ones, sq, _NT, preferred_element_type=jnp.float32)
        e = jnp.exp(proj * scale - ssq * (0.5 * scale * scale))
        return (e * inv_sqrt_m + 1e-6).astype(jnp.bfloat16)

    def finalize(h):
        q = jnp.broadcast_to(qb[h], (m, d)).astype(jnp.float32)
        proj = jnp.sum(q * omb[...].astype(jnp.float32), axis=1, keepdims=True)
        ssq = jnp.sum(q * q, axis=1, keepdims=True)
        phi_q = jnp.exp(proj * scale - ssq * (0.5 * scale * scale)) * inv_sqrt_m + 1e-6
        num = jnp.sum(phi_q * kv_acc[...], axis=0, keepdims=True)
        z = jnp.sum(z_acc[...], axis=1, keepdims=True)
        den = jnp.sum(phi_q * z, axis=0, keepdims=True) + 1e-6
        o_ref[h] = (num / den).astype(o_ref.dtype)
        kv_acc[...] = jnp.zeros_like(kv_acc)
        z_acc[...] = jnp.zeros_like(z_acc)

    def body(i, _):
        slot = lax.rem(i, _SLOTS)
        nxt = i + _SLOTS - 1

        @pl.when(nxt < n_chunks)
        def _():
            start(nxt, lax.rem(nxt, _SLOTS))

        wait(kb, 0, slot)
        phi = phi_k(kb[slot])
        phi32 = phi.astype(jnp.float32)
        z = phi32[:, 0:128]
        for c in range(128, _CHUNK, 128):
            z = z + phi32[:, c:c + 128]
        z_acc[...] += z
        wait(vb, 1, slot)
        kv_acc[...] += jnp.dot(phi, vb[slot], preferred_element_type=jnp.float32)

        @pl.when(lax.rem(i, per_head) == per_head - 1)
        def _():
            finalize(i // per_head)

        return 0

    lax.fori_loop(0, n_chunks, body, 0)


@jax.jit
def pallas_standalone__linear_kernel_rfa__decode_kernel(
    q: jax.Array,
    k: jax.Array,
    v: jax.Array,
    omega: jax.Array,
):
    b, h, sq, d = q.shape
    sk = k.shape[2]
    m = omega.shape[0]
    assert sq == 1 and sk % _CHUNK == 0 and d % 256 == 0 and m % 16 == 0
    hbm = pl.BlockSpec(memory_space=pl.ANY)
    out = pl.pallas_call(
        functools.partial(_kernel, sk=sk),
        in_specs=[hbm] * 4,
        out_specs=pl.BlockSpec(memory_space=pltpu.VMEM),
        out_shape=jax.ShapeDtypeStruct((b * h, sq, d), q.dtype),
        scratch_shapes=[
            pltpu.VMEM((_SLOTS, _CHUNK, d), k.dtype),
            pltpu.VMEM((_SLOTS, _CHUNK, d), v.dtype),
            pltpu.VMEM((b * h, sq, d), q.dtype),
            pltpu.VMEM((m, d), omega.dtype),
            pltpu.VMEM((m, d), jnp.float32),
            pltpu.VMEM((m, 128), jnp.float32),
            pltpu.SemaphoreType.DMA((2, _SLOTS)),
            pltpu.SemaphoreType.DMA((2,)),
        ],
        compiler_params=pltpu.CompilerParams(vmem_limit_bytes=48 * 1024 * 1024),
    )(q.reshape(b * h, sq, d), omega, k.reshape(b * h * sk, d), v.reshape(b * h * sk, d))
    return out.reshape(b, h, sq, d)
```

```python
import functools

import jax
import jax.numpy as jnp
from jax import lax
import jax.experimental.pallas as pl
import jax.experimental.pallas.tpu as pltpu

_NT = (((1,), (1,)), ((), ()))

_CHUNK = 1024
_SLOTS = 6
_DMA_ROWS = 96
_PIECES = tuple((o, min(_DMA_ROWS, _CHUNK - o)) for o in range(0, _CHUNK, _DMA_ROWS))


def _kernel(q_hbm, om_hbm, k_hbm, v_hbm, o_ref,
            kb, vb, qb, omb, kv_acc, z_acc, o_acc, sems, sem_in, *, sk):
    n_rows, d = k_hbm.shape
    m = omb.shape[0]
    dt, f32 = kb.dtype, jnp.float32
    scale = float(d) ** -0.25
    inv_sqrt_m = float(m) ** -0.5
    n_chunks = n_rows // _CHUNK
    per_head = sk // _CHUNK

    def rnd(x):
        return x.astype(dt).astype(f32)

    def start(i, slot):
        for o, n in _PIECES:
            src, dst = pl.ds(i * _CHUNK + o, n), pl.ds(o, n)
            pltpu.make_async_copy(
                k_hbm.at[src], kb.at[slot, dst], sems.at[0, slot]).start(priority=0)
            pltpu.make_async_copy(
                v_hbm.at[src], vb.at[slot, dst], sems.at[1, slot]).start(priority=1)

    def wait(buf, which, slot):
        pltpu.make_async_copy(buf.at[slot], buf.at[slot], sems.at[which, slot]).wait()

    def features(x):
        proj = lax.dot_general(omb[...], x, _NT, preferred_element_type=f32) * scale
        lo = x[:, : d // 2].astype(f32)
        hi = x[:, d // 2:].astype(f32)
        sq = (lo * lo + hi * hi).astype(dt)
        ones = jnp.ones((m, d // 2), dt)
        half_sq = lax.dot_general(ones, sq, _NT, preferred_element_type=f32) * (0.5 * scale * scale)
        e = rnd(jnp.exp(rnd(rnd(proj) - rnd(half_sq))))
        return (rnd(e * inv_sqrt_m) + 1e-6).astype(dt)

    for i in range(_SLOTS - 1):
        start(i, i)
    om_copy = pltpu.make_async_copy(om_hbm, omb, sem_in.at[0])
    q_copy = pltpu.make_async_copy(q_hbm, qb, sem_in.at[1])
    om_copy.start()
    q_copy.start()
    kv_acc[...] = jnp.zeros_like(kv_acc)
    z_acc[...] = jnp.zeros_like(z_acc)
    o_acc[...] = jnp.zeros_like(o_acc)
    om_copy.wait()
    q_copy.wait()
    phi_q_all = features(qb[...]).astype(f32)

    def finalize(h):
        col = lax.broadcasted_iota(jnp.int32, phi_q_all.shape, 1)
        phi_q = jnp.sum(jnp.where(col == h, phi_q_all, 0.0), axis=1, keepdims=True)
        num = rnd(jnp.sum(phi_q * rnd(kv_acc[...]), axis=0, keepdims=True))
        z = rnd(jnp.sum(z_acc[...], axis=1, keepdims=True))
        den = rnd(rnd(jnp.sum(phi_q * z, axis=0, keepdims=True)) + 1e-6)
        row = lax.broadcasted_iota(jnp.int32, o_acc.shape, 0)
        o_acc[...] = jnp.where(row == h, num / den, o_acc[...])
        kv_acc[...] = jnp.zeros_like(kv_acc)
        z_acc[...] = jnp.zeros_like(z_acc)

    def body(i, carry):
        slot = lax.rem(i, _SLOTS)
        nxt = i + _SLOTS - 1

        @pl.when(nxt < n_chunks)
        def _():
            start(nxt, lax.rem(nxt, _SLOTS))

        wait(kb, 0, slot)
        phi_k = features(kb[slot])
        phi_f = phi_k.astype(f32)
        z = phi_f[:, 0:128]
        for c in range(128, _CHUNK, 128):
            z = z + phi_f[:, c:c + 128]
        z_acc[...] += z
        wait(vb, 1, slot)
        kv_acc[...] += jnp.dot(phi_k, vb[slot], preferred_element_type=f32)

        @pl.when(lax.rem(i, per_head) == per_head - 1)
        def _():
            finalize(i // per_head)

        return carry

    lax.fori_loop(0, n_chunks, body, 0)
    o_ref[...] = o_acc[...].astype(o_ref.dtype)


@jax.jit
def pallas_standalone__linear_kernel_rfa__decode_kernel(
    q: jax.Array,
    k: jax.Array,
    v: jax.Array,
    omega: jax.Array,
):
    b, h, sq, d = q.shape
    sk = k.shape[2]
    m = omega.shape[0]
    assert sq == 1 and sk % _CHUNK == 0 and d == 256 and m % 16 == 0
    assert b * h * sk // _CHUNK >= _SLOTS
    hbm = pl.BlockSpec(memory_space=pl.ANY)
    out = pl.pallas_call(
        functools.partial(_kernel, sk=sk),
        in_specs=[hbm] * 4,
        out_specs=pl.BlockSpec(memory_space=pltpu.VMEM),
        out_shape=jax.ShapeDtypeStruct((b * h, d), q.dtype),
        scratch_shapes=[
            pltpu.VMEM((_SLOTS, _CHUNK, d), k.dtype),
            pltpu.VMEM((_SLOTS, _CHUNK, d), v.dtype),
            pltpu.VMEM((b * h, d), q.dtype),
            pltpu.VMEM((m, d), omega.dtype),
            pltpu.VMEM((m, d), jnp.float32),
            pltpu.VMEM((m, 128), jnp.float32),
            pltpu.VMEM((b * h, d), jnp.float32),
            pltpu.SemaphoreType.DMA((2, _SLOTS)),
            pltpu.SemaphoreType.DMA((2,)),
        ],
        compiler_params=pltpu.CompilerParams(vmem_limit_bytes=32 * 1024 * 1024),
    )(q.reshape(b * h, d), omega, k.reshape(b * h * sk, d), v.reshape(b * h * sk, d))
    return out.reshape(b, h, sq, d)
```
